```python
import os as _os
_os.environ.setdefault("JAX_PLATFORMS", "cpu")
import jax
import jax.numpy as jnp

def _softmax(x, axis=-1):
    return jax.nn.softmax(x, axis=axis)
def _gelu(x):
    return jax.nn.gelu(x, approximate=True)
def _silu(x):
    return jax.nn.silu(x)
def _sigmoid(x):
    return jax.nn.sigmoid(x)
def _layernorm(x, axis=-1, eps=1e-5):
    m = jnp.mean(x, axis=axis, keepdims=True)
    v = jnp.var(x, axis=axis, keepdims=True)
    return (x - m) / jnp.sqrt(v + eps)
def _scatter_add(tgt, idx, src, axis=0):
    return tgt.at[idx].add(src)
def _segment_sum(src, seg, n):
    return jax.ops.segment_sum(src, seg, n)
class _Rng:
    def __init__(self, key):
        self._k = key
    def _next(self):
        self._k, sub = jax.random.split(self._k)
        return sub
    def normal(self, shape):
        return jax.random.normal(self._next(), shape, dtype=jnp.bfloat16)
    def randint(self, lo, hi, shape):
        return jax.random.randint(self._next(), shape, lo, hi, dtype=jnp.int32)
    def uniform(self, shape, lo=0.0, hi=1.0):
        return jax.random.uniform(self._next(), shape, jnp.bfloat16, lo, hi)
    def permutation(self, n):
        return jax.random.permutation(self._next(), n)


kernel_name = 'standalone__gqa_softmax__near_ridge'

def setup_inputs():
    _rng = _Rng(jax.random.key(int.from_bytes(__import__("os").urandom(4), "little")))
    _w = (lambda a: (lambda t: t.astype(jnp.bfloat16) if jnp.issubdtype(t.dtype, jnp.floating) else t)(jnp.asarray(a)))
    B, Hq, Hkv, Sq, Sk, D = 8, 32, 8, 112, 2048, 128
    return {
        "q": _w((lambda *s: _rng.normal(s) * 0.4)(B, Hq, Sq, D)),
        "k": _w((lambda *s: _rng.normal(s) * 0.4)(B, Hkv, Sk, D)),
        "v": _w((lambda *s: _rng.normal(s) * 0.05)(B, Hkv, Sk, D)),
    }

def reference(q, k, v):
    B, Hq, Sq, D = q.shape
    Hkv = k.shape[1]
    rep = Hq // Hkv
    k = jnp.repeat(k, rep, axis=1)
    v = jnp.repeat(v, rep, axis=1)
    scale = D ** -0.5
    scores = jnp.einsum("bhqd,bhkd->bhqk", q, k) * scale
    p = _softmax(scores, axis=-1)
    return jnp.einsum("bhqk,bhkd->bhqd", p, v)
```

```python
import jax
import jax.numpy as jnp
import jax.experimental.pallas as pl
import jax.experimental.pallas.tpu as pltpu

LOG2E = 1.4426950408889634
NT = (((1,), (1,)), ((), ()))


@jax.jit
def pallas_standalone__gqa_softmax__near_ridge_kernel(
    q: jax.Array,
    k: jax.Array,
    v: jax.Array,
):
    B, Hq, Sq, D = q.shape
    Hkv, Sk = k.shape[1], k.shape[2]
    rep = Hq // Hkv
    M = rep * Sq
    NP = B * Hkv
    R = 64
    NA, G, AH = 4, 4, 1
    n = M // R
    NIT = (NP - NA) // G
    NX = NP + AH * G
    c = (D ** -0.5) * LOG2E

    q3 = q.reshape(NP, M, D)
    k3 = k.reshape(NP, Sk, D)
    v3 = v.reshape(NP, Sk, D)

    def kern(q_hbm, k_hbm, v_hbm, o_hbm, qbuf, kbuf, vbuf, obuf, asem, bsem, osem):
        def copies(src0, dst0, cnt, sem, r):
            return (pltpu.make_async_copy(q_hbm.at[pl.ds(src0, cnt)], qbuf.at[pl.ds(dst0, cnt)], sem.at[0, r]),
                    pltpu.make_async_copy(k_hbm.at[pl.ds(src0, cnt)], kbuf.at[pl.ds(dst0, cnt)], sem.at[1, r]),
                    pltpu.make_async_copy(v_hbm.at[pl.ds(src0, cnt)], vbuf.at[pl.ds(dst0, cnt)], sem.at[2, r]))

        def out_copy(p0, cnt, r):
            return pltpu.make_async_copy(obuf.at[pl.ds(p0, cnt)], o_hbm.at[pl.ds(p0, cnt)], osem.at[r])

        def qk(p, i):
            return jax.lax.dot_general(qbuf[p, i * R:(i + 1) * R, :], kbuf[p], NT,
                                       preferred_element_type=jnp.float32)

        def softmax(s):
            m = jnp.max(s, axis=-1, keepdims=True)
            p = jnp.exp2((s - m) * c)
            l = jnp.sum(p, axis=-1, keepdims=True)
            return p.astype(jnp.bfloat16), l

        def pv(p, l, pr, i):
            o = jnp.dot(p, vbuf[pr], preferred_element_type=jnp.float32)
            o = o * pltpu.reciprocal(l, approx=True)
            obuf[pr, i * R:(i + 1) * R, :] = o.astype(obuf.dtype)

        def region(p0, gn):
            N = n * gn
            s = qk(p0, 0)
            for j in range(N):
                s_next = qk(p0 + (j + 1) // n, (j + 1) % n) if j + 1 < N else None
                pp, l = softmax(s)
                pv(pp, l, p0 + j // n, j % n)
                s = s_next

        for j in range(NA):
            for cp in copies(j, j, 1, asem, j):
                cp.start()
        for r in range(AH):
            for cp in copies(NA + r * G, NA + r * G, G, bsem, r):
                cp.start()

        def body_a(j, carry):
            for cp in copies(j, j, 1, asem, j):
                cp.wait()
            region(j, 1)
            return carry

        jax.lax.fori_loop(0, NA, body_a, 0)
        out_copy(0, NA, NIT).start()

        def body_b(it, carry):
            p0 = NA + it * G
            for cp in copies(p0, p0, G, bsem, it):
                cp.wait()
            nx = p0 + AH * G
            for cp in copies(jnp.minimum(nx, NP - G), nx, G, bsem, it + AH):
                cp.start()
            region(p0, G)
            out_copy(p0, G, it).start()
            return carry

        jax.lax.fori_loop(0, NIT, body_b, 0)
        for r in range(AH):
            for cp in copies(NP - G, NP + r * G, G, bsem, NIT + r):
                cp.wait()
        out_copy(0, NA, NIT).wait()

        def body_w(it, carry):
            out_copy(NA + it * G, G, it).wait()
            return carry

        jax.lax.fori_loop(0, NIT, body_w, 0)

    out = pl.pallas_call(
        kern,
        in_specs=[pl.BlockSpec(memory_space=pl.ANY)] * 3,
        out_specs=pl.BlockSpec(memory_space=pl.ANY),
        out_shape=jax.ShapeDtypeStruct((NP, M, D), q.dtype),
        scratch_shapes=[
            pltpu.VMEM((NX, M, D), q.dtype),
            pltpu.VMEM((NX, Sk, D), k.dtype),
            pltpu.VMEM((NX, Sk, D), v.dtype),
            pltpu.VMEM((NP, M, D), q.dtype),
            pltpu.SemaphoreType.DMA((3, NA)),
            pltpu.SemaphoreType.DMA((3, NIT + AH)),
            pltpu.SemaphoreType.DMA((NIT + 1,)),
        ],
        compiler_params=pltpu.CompilerParams(vmem_limit_bytes=110 * 1024 * 1024),
    )(q3, k3, v3)
    return out.reshape(B, Hq, Sq, D)
```

```python
import jax
import jax.numpy as jnp
import jax.experimental.pallas as pl
import jax.experimental.pallas.tpu as pltpu

LOG2E = 1.4426950408889634
NT = (((1,), (1,)), ((), ()))
G = 7
PD = 3
R = 64
sp = 1


@jax.jit
def pallas_standalone__gqa_softmax__near_ridge_kernel(
    q: jax.Array,
    k: jax.Array,
    v: jax.Array,
):
    B, Hq, Sq, D = q.shape
    Hkv, Sk = k.shape[1], k.shape[2]
    M = (Hq // Hkv) * Sq
    NP = B * Hkv
    q3 = q.reshape(NP, M, D); k3 = k.reshape(NP, Sk, D); v3 = v.reshape(NP, Sk, D)
    c = (D ** -0.5) * LOG2E
    n = M // R
    NIT = NP // G
    REM = NP - NIT * G
    NX = NP + PD
    def kern(q_hbm, k_hbm, v_hbm, o_hbm, buf, obuf, isem, osem):
        K0 = M; V0 = M + Sk
        def copies(src, dst):
            return (pltpu.make_async_copy(q_hbm.at[src], buf.at[dst, pl.ds(0, M)], isem.at[dst]),
                    pltpu.make_async_copy(k_hbm.at[src], buf.at[dst, pl.ds(K0, Sk)], isem.at[dst]),
                    pltpu.make_async_copy(v_hbm.at[src], buf.at[dst, pl.ds(V0, Sk)], isem.at[dst]))
        def wait_all(dst):
            pltpu.make_async_copy(buf.at[dst], buf.at[dst], isem.at[dst]).wait()
        def out_copy(p):
            return pltpu.make_async_copy(obuf.at[p], o_hbm.at[p], osem.at[p])
        def qk(p, i):
            return jax.lax.dot_general(buf[p, i*R:(i+1)*R, :], buf[p, K0:K0+Sk, :], NT, preferred_element_type=jnp.float32)
        def sm(s):
            m = jnp.max(s, axis=-1, keepdims=True)
            p = jnp.exp2((s - m) * c)
            l = jnp.sum(p, axis=-1, keepdims=True)
            return p.astype(jnp.bfloat16), l
        def pv(p, l, pr, i):
            o = jnp.dot(p, buf[pr, V0:V0+Sk, :], preferred_element_type=jnp.float32)
            o = o * pltpu.reciprocal(l, approx=True)
            obuf[pr, i*R:(i+1)*R, :] = o.astype(jnp.bfloat16)
        def region(p0, Gn):
            N = n * Gn
            wait_all(p0)
            s = qk(p0, 0)
            for j in range(N):
                g, i = divmod(j, n)
                g1, i1 = divmod(j + 1, n)
                if j + 1 < N:
                    if i1 == 0:
                        wait_all(p0 + g1)
                    s_next = qk(p0 + g1, i1)
                else:
                    s_next = None
                pp, l = sm(s)
                pv(pp, l, p0 + g, i)
                s = s_next
                if i == sp - 1:
                    nx = p0 + g + PD
                    for cp in copies(jnp.minimum(nx, NP - 1), nx): cp.start()
                if i == n - 1:
                    out_copy(p0 + g).start()
        for j in range(PD):
            for cp in copies(j, j): cp.start()
        def body(it, cr):
            region(it * G, G)
            return cr
        jax.lax.fori_loop(0, NIT, body, 0)
        if REM: region(NIT * G, REM)
        for r in range(PD):
            wait_all(NP + r)
        def bodyW(p, cr):
            out_copy(p).wait()
            return cr
        jax.lax.fori_loop(0, NP, bodyW, 0)
    kw = dict(vmem_limit_bytes=110 * 1024 * 1024)
    kw["flags"] = {"XLA_TPU_RESCHEDULE_DMA_DONES": True}
    out = pl.pallas_call(kern,
        in_specs=[pl.BlockSpec(memory_space=pl.ANY)] * 3,
        out_specs=pl.BlockSpec(memory_space=pl.ANY),
        out_shape=jax.ShapeDtypeStruct((NP, M, D), q.dtype),
        scratch_shapes=[pltpu.VMEM((NX, M + 2 * Sk, D), q.dtype),
                        pltpu.VMEM((NP, M, D), q.dtype),
                        pltpu.SemaphoreType.DMA((NX,)), pltpu.SemaphoreType.DMA((NP,))],
        compiler_params=pltpu.CompilerParams(**kw),
    )(q3, k3, v3)
    return out.reshape(B, Hq, Sq, D)
```

```python
import jax
import jax.numpy as jnp
import jax.experimental.pallas as pl
import jax.experimental.pallas.tpu as pltpu

LOG2E = 1.4426950408889634
NT = (((1,), (1,)), ((), ()))
R = 64
G = 7
PD = 3
NS = 4


@jax.jit
def pallas_standalone__gqa_softmax__near_ridge_kernel(
    q: jax.Array,
    k: jax.Array,
    v: jax.Array,
):
    B, Hq, Sq, D = q.shape
    Hkv, Sk = k.shape[1], k.shape[2]
    M = (Hq // Hkv) * Sq
    NP = B * Hkv
    n = M // R
    first = NP % G
    NIT = NP // G
    assert M % R == 0 and first >= 1 and PD < NS
    K0, V0 = M, M + Sk
    c = (D ** -0.5) * LOG2E

    def kern(q_hbm, k_hbm, v_hbm, o_hbm, buf, obuf, isem, vsem, osem):
        def copies(src, dst, sv=None):
            sem = isem.at[dst % NS]
            return (
                pltpu.make_async_copy(q_hbm.at[src], buf.at[dst, pl.ds(0, M)], sem),
                pltpu.make_async_copy(k_hbm.at[src], buf.at[dst, pl.ds(K0, Sk)], sem),
                pltpu.make_async_copy(v_hbm.at[src], buf.at[dst, pl.ds(V0, Sk)],
                                      sem if sv is None else sv),
            )

        def wait_pair(dst):
            pltpu.make_async_copy(buf.at[dst], buf.at[dst], isem.at[dst % NS]).wait()

        def qk(p, i):
            return jax.lax.dot_general(
                buf[p, i * R:(i + 1) * R, :], buf[p, K0:K0 + Sk, :], NT,
                preferred_element_type=jnp.float32)

        def softmax(s):
            m = jnp.max(s, axis=-1, keepdims=True)
            p = jnp.exp2((s - m) * c)
            l = jnp.sum(p, axis=-1, keepdims=True)
            return p.astype(jnp.bfloat16), l

        def pv(p, l, pr, i):
            o = jnp.dot(p, buf[pr, V0:V0 + Sk, :], preferred_element_type=jnp.float32)
            o = o * pltpu.reciprocal(l, approx=True)
            obuf[pr, i * R:(i + 1) * R, :] = o.astype(obuf.dtype)

        def region(p0, gn, is_first=False):
            N = n * gn
            if is_first:
                qk0 = buf.at[0, pl.ds(0, V0)]
                pltpu.make_async_copy(qk0, qk0, isem.at[0]).wait()
            else:
                wait_pair(p0)
            s = qk(p0, 0)
            for j in range(N):
                g, i = divmod(j, n)
                g1, i1 = divmod(j + 1, n)
                s_next = None
                if j + 1 < N:
                    if i1 == 0:
                        wait_pair(p0 + g1)
                    s_next = qk(p0 + g1, i1)
                pp, l = softmax(s)
                if is_first and j == 0:
                    copies(0, 0, vsem.at[0])[2].wait()
                pv(pp, l, p0 + g, i)
                s = s_next
                if i == 0:
                    nx = p0 + g + PD
                    for cp in copies(jnp.minimum(nx, NP - 1), nx):
                        cp.start()
                if i == n - 1:
                    pltpu.make_async_copy(obuf.at[p0 + g], o_hbm.at[p0 + g], osem.at[0]).start()

        for cp in copies(0, 0, vsem.at[0]):
            cp.start()
        for j in range(1, PD):
            for cp in copies(j, j):
                cp.start()
        region(0, first, True)

        def body(it, carry):
            region(first + it * G, G)
            return carry

        jax.lax.fori_loop(0, NIT, body, 0)
        for r in range(PD):
            wait_pair(NP + r)
        pltpu.make_async_copy(obuf, o_hbm, osem.at[0]).wait()

    out = pl.pallas_call(
        kern,
        in_specs=[pl.BlockSpec(memory_space=pl.ANY)] * 3,
        out_specs=pl.BlockSpec(memory_space=pl.ANY),
        out_shape=jax.ShapeDtypeStruct((NP, M, D), q.dtype),
        scratch_shapes=[
            pltpu.VMEM((NP + PD, M + 2 * Sk, D), q.dtype),
            pltpu.VMEM((NP, M, D), q.dtype),
            pltpu.SemaphoreType.DMA((NS,)),
            pltpu.SemaphoreType.DMA((1,)),
            pltpu.SemaphoreType.DMA((1,)),
        ],
        compiler_params=pltpu.CompilerParams(
            vmem_limit_bytes=110 * 1024 * 1024,
            flags={"XLA_TPU_RESCHEDULE_DMA_DONES": True},
        ),
    )(q.reshape(NP, M, D), k.reshape(NP, Sk, D), v.reshape(NP, Sk, D))
    return out.reshape(B, Hq, Sq, D)
```
